```python
import os as _os
_os.environ.setdefault("JAX_PLATFORMS", "cpu")
import jax
import jax.numpy as jnp

def _softmax(x, axis=-1):
    return jax.nn.softmax(x, axis=axis)
def _gelu(x):
    return jax.nn.gelu(x, approximate=True)
def _silu(x):
    return jax.nn.silu(x)
def _sigmoid(x):
    return jax.nn.sigmoid(x)
def _layernorm(x, axis=-1, eps=1e-5):
    m = jnp.mean(x, axis=axis, keepdims=True)
    v = jnp.var(x, axis=axis, keepdims=True)
    return (x - m) / jnp.sqrt(v + eps)
def _scatter_add(tgt, idx, src, axis=0):
    return tgt.at[idx].add(src)
def _segment_sum(src, seg, n):
    return jax.ops.segment_sum(src, seg, n)
class _Rng:
    def __init__(self, key):
        self._k = key
    def _next(self):
        self._k, sub = jax.random.split(self._k)
        return sub
    def normal(self, shape):
        return jax.random.normal(self._next(), shape, dtype=jnp.bfloat16)
    def randint(self, lo, hi, shape):
        return jax.random.randint(self._next(), shape, lo, hi, dtype=jnp.int32)
    def uniform(self, shape, lo=0.0, hi=1.0):
        return jax.random.uniform(self._next(), shape, jnp.bfloat16, lo, hi)
    def permutation(self, n):
        return jax.random.permutation(self._next(), n)


kernel_name = 'recurrent_scan__ssm_conv_s5__mixer_s_mlp__prompt'

def setup_inputs():
    _rng = _Rng(jax.random.key(int.from_bytes(__import__("os").urandom(4), "little")))
    _w = (lambda a: (lambda t: t.astype(jnp.bfloat16) if jnp.issubdtype(t.dtype, jnp.floating) else t)(jnp.asarray(a)))
    def _A_setup():
        B, S, D = 1, 2048, 640
        P = D
        Lambda_re = -0.5 * jnp.exp((lambda *s: _rng.normal(s) * 0.8)(P))
        Lambda_im = (lambda *s: _rng.normal(s) * 0.8)(P) * 1.0
        B_re = (lambda *s: _rng.normal(s) * 0.8)(P, D) * (D ** -0.5)
        B_im = (lambda *s: _rng.normal(s) * 0.8)(P, D) * (D ** -0.5)
        C_re = (lambda *s: _rng.normal(s) * 0.8)(D, P) * (P ** -0.5)
        C_im = (lambda *s: _rng.normal(s) * 0.8)(D, P) * (P ** -0.5)
        log_dt = (lambda *s: _rng.normal(s) * 0.8)(P) * 0.3 - 2.0
        Dskip = (lambda *s: _rng.normal(s) * 0.8)(D)
        return {
            "x": _w((lambda *s: _rng.normal(s) * 0.05)(B, S, D)),
            "Lambda_re": _w(Lambda_re),
            "Lambda_im": _w(Lambda_im),
            "B_re": _w(B_re),
            "B_im": _w(B_im),
            "C_re": _w(C_re),
            "C_im": _w(C_im),
            "log_dt": _w(log_dt),
            "Dskip": _w(Dskip),
        }
    _A_in = _A_setup()

    def _B_setup():
        B, S, D, F = 1, 2048, 640, 1536
        return {
            "x":  _w((lambda *s: _rng.normal(s) * 0.05)(B, S, D)),
            "w1": _w((lambda *s: _rng.normal(s) * 0.8)(D, D) * (D ** -0.5)),
            "w2": _w((lambda *s: _rng.normal(s) * 0.8)(D, D) * (D ** -0.5)),
            "w3": _w((lambda *s: _rng.normal(s) * 0.8)(D, F) * (D ** -0.5)),
            "w4": _w((lambda *s: _rng.normal(s) * 0.8)(F, D) * (F ** -0.5)),
        }
    _B_in = _B_setup()

    return {
        "A_x": _A_in["x"],
        "A_Lambda_re": _A_in["Lambda_re"],
        "A_Lambda_im": _A_in["Lambda_im"],
        "A_B_re": _A_in["B_re"],
        "A_B_im": _A_in["B_im"],
        "A_C_re": _A_in["C_re"],
        "A_C_im": _A_in["C_im"],
        "A_log_dt": _A_in["log_dt"],
        "A_Dskip": _A_in["Dskip"],
        "B_x": _B_in["x"],
        "B_w1": _B_in["w1"],
        "B_w2": _B_in["w2"],
        "B_w3": _B_in["w3"],
        "B_w4": _B_in["w4"],
    }

def reference(A_x, A_Lambda_re, A_Lambda_im, A_B_re, A_B_im, A_C_re, A_C_im, A_log_dt, A_Dskip, B_x, B_w1, B_w2, B_w3, B_w4):
    def _A_ref(x, Lambda_re, Lambda_im, B_re, B_im, C_re, C_im, log_dt, Dskip):
        Bsz, L, H = x.shape
        Lam = Lambda_re + 1j * Lambda_im
        Bmat = B_re + 1j * B_im
        Cmat = C_re + 1j * C_im
        dt = jnp.exp(log_dt)
        Lam_bar = jnp.exp(dt * Lam)
        B_bar = ((Lam_bar - 1.0) / Lam)[:, None] * Bmat
        Bu = jnp.einsum("bld,pd->blp", x + 0j, B_bar)
        h = jnp.zeros_like(Bu[:, 0, :])
        hs = []
        for t in range(L):
            h = Lam_bar[None, :] * h + Bu[:, t, :]
            hs.append(h)
        hseq = jnp.stack(hs, 1)
        y = 2.0 * jnp.einsum("blp,dp->bld", hseq, Cmat).real + x * Dskip[None, None, :]
        return y

    def _B_ref(x, w1, w2, w3, w4):
        B, S, D = x.shape
        h = _gelu(_layernorm(x, axis=-1) @ w1)
        c = D // 4
        g0 = jnp.pad(h[:, :, 0*c:1*c], ((0, 0), (1, 0), (0, 0)))[:, :S, :]
        g1 = jnp.pad(h[:, :, 1*c:2*c], ((0, 0), (0, 1), (0, 0)))[:, 1:, :]
        g2 = jnp.pad(h[:, :, 2*c:3*c], ((0, 0), (2, 0), (0, 0)))[:, :S, :]
        g3 = jnp.pad(h[:, :, 3*c:   ], ((0, 0), (0, 2), (0, 0)))[:, 2:, :]
        hs = jnp.concatenate([g0, g1, g2, g3], axis=-1) @ w2
        x1 = x + hs
        h2 = _gelu(_layernorm(x1, axis=-1) @ w3) @ w4
        return x1 + h2

    x = A_x
    xn = _layernorm(x, axis=-1)
    s = _A_ref(xn, A_Lambda_re, A_Lambda_im, A_B_re, A_B_im, A_C_re, A_C_im, A_log_dt, A_Dskip)
    g = _silu(_B_ref(xn, B_w1, B_w2, B_w3, B_w4))
    return x + s * g
```

```python
import numpy as np
import jax
import jax.numpy as jnp
from jax import lax
from jax.experimental import pallas as pl
from jax.experimental.pallas import tpu as pltpu

S, D, P, F = 2048, 640, 640, 1536
NS = 8
L = S // NS
EPS = 1e-5
f32, bf16 = jnp.float32, jnp.bfloat16
C0 = 0.7978845608028654
C1 = 0.044715
NTD = (((1,), (1,)), ((), ()))

P2 = dict(
    D=['m3', 'scan2', 'gsel+', 'm2+', 'm4', 'ln2+', 'mc', 'fin', 'ost'],
    G=['m3c', 'scan2', 'gsel+', 'm2+', 'outc', 'ln2+', 'ost'],
    I=['m3c', 'scan2', 'outc0', 'gsel+', 'm2+', 'outc1', 'ln2+', 'outc2', 'outc3', 'outc4', 'ost'],
    J=['m3c', 'scan2', 'outc0', 'outc1', 'gsel+', 'm2+', 'ln2+', 'outc2', 'outc3', 'outc4', 'ost'],
)

def default_prog(NT, cfg):
    prog = []
    A = prog.append
    V = ('lre', 'lim', 'ldt', 'dsk')
    last = 'x%d' % (NT - 1)
    start = cfg.get('start', 1)
    if start == 1:
        A(('S', 'x0', '|', 'bre', '|', 'bim', '|', last, '|', 'w1', '|', 'x1') + V)
        A(('W', 'x0')); A(('ln1', 0))
        A(('W', 'bre')); A(('mbre', 0))
        A(('W', 'bim', last)); A(('S', 'x2', 'x3')); A(('ln1', NT - 1)); A(('mbim', 0))
        A(('W', 'w1', 'x1') + V); A(('S', 'cre', 'cim') + tuple('x%d' % k for k in range(4, NT - 1))); A(('lam',)); A(('mw1', NT - 1))
        A(('ln1', 1))
        A(('stu', 0)); A(('scan1', 0)); A(('gelu1', NT - 1))
        i0 = 1
    elif start == 2:
        A(('S', 'x0', '|', 'bre', '|', 'x1', '|', 'bim', '|', last, '|', 'w1') + V)
        A(('W', 'x0')); A(('ln1', 0))
        A(('W', 'bre')); A(('mbre', 0))
        A(('W', 'x1')); A(('ln1', 1)); A(('mbre', 1))
        A(('W', 'bim', last)); A(('S', 'x2', 'x3')); A(('ln1', NT - 1)); A(('mbim', 0)); A(('mbim', 1))
        A(('W', 'w1') + V); A(('S', 'cre', 'cim') + tuple('x%d' % k for k in range(4, NT - 1))); A(('lam',)); A(('mw1', NT - 1))
        A(('stu', 0)); A(('scan1', 0)); A(('gelu1', NT - 1))
        A(('W', 'x2', 'x3')); A(('ln1', 2)); A(('mw1', 0))
        A(('stu', 1)); A(('scan1', 1)); A(('gelu1', 0))
        i0 = 2
    elif start == 4:
        sp = cfg.get('sp', 2)
        A(('S', 'x0', '|', 'bre', '|', 'x1', '|', 'x2', '|', 'bim', '|', last, '|', 'w1') + V)
        A(('W', 'x0')); A(('ln1', 0))
        A(('W', 'bre')); A(('mbreP', 0, 0, sp)); A(('W', 'x1')); A(('ln1', 1)); A(('mbreP', 0, sp, 5))
        A(('mbreP', 1, 0, sp)); A(('W', 'x2')); A(('ln1', 2)); A(('mbreP', 1, sp, 5)); A(('mbre', 2))
        A(('W', 'bim', last)); A(('S', 'x3', 'x4')); A(('ln1', NT - 1)); A(('mbim', 0)); A(('mbim', 1)); A(('mbim', 2))
        A(('W', 'w1') + V); A(('S', 'cre', 'cim') + tuple('x%d' % k for k in range(5, NT - 1))); A(('lam',)); A(('mw1', NT - 1))
        A(('stu', 0)); A(('scan1', 0)); A(('gelu1', NT - 1))
        A(('W', 'x3', 'x4')); A(('ln1', 3)); A(('mw1', 0))
        A(('stu', 1)); A(('scan1', 1)); A(('gelu1', 0))
        A(('mw1', 1)); A(('stu', 2)); A(('scan1', 2)); A(('gelu1', 1))
        i0 = 3
    elif start == 5:
        A(('S', 'x0', '|', 'x1', '|', 'x2', '|', 'bre', '|', 'bim', '|', last, '|', 'w1') + V)
        A(('W', 'x0')); A(('ln1', 0)); A(('W', 'x1')); A(('ln1', 1)); A(('W', 'x2')); A(('ln1', 2))
        A(('W', 'bre')); A(('mbre', 0)); A(('mbre', 1)); A(('mbre', 2))
        A(('W', 'bim', last)); A(('S', 'x3', 'x4')); A(('ln1', NT - 1)); A(('mbim', 0)); A(('mbim', 1)); A(('mbim', 2))
        A(('W', 'w1') + V); A(('S', 'cre', 'cim') + tuple('x%d' % k for k in range(5, NT - 1))); A(('lam',)); A(('mw1', NT - 1))
        A(('stu', 0)); A(('scan1', 0)); A(('gelu1', NT - 1))
        A(('W', 'x3', 'x4')); A(('ln1', 3)); A(('mw1', 0))
        A(('stu', 1)); A(('scan1', 1)); A(('gelu1', 0))
        A(('mw1', 1)); A(('stu', 2)); A(('scan1', 2)); A(('gelu1', 1))
        i0 = 3
    elif start == 6:
        A(('S', 'x0', '|', 'x1', '|', 'bre', '|', 'bim', '|', last, '|', 'w1') + V)
        A(('W', 'x0')); A(('ln1', 0)); A(('W', 'x1')); A(('ln1', 1))
        A(('W', 'bre')); A(('S', 'x2', 'x3')); A(('mbre', 0)); A(('mbre', 1))
        A(('W', 'bim', last)); A(('ln1', NT - 1)); A(('mbim', 0)); A(('mbim', 1))
        A(('W', 'w1') + V); A(('S', 'cre', 'cim') + tuple('x%d' % k for k in range(4, NT - 1))); A(('lam',)); A(('mw1', NT - 1))
        A(('stu', 0)); A(('scan1', 0)); A(('gelu1', NT - 1))
        A(('W', 'x2', 'x3')); A(('ln1', 2)); A(('mw1', 0))
        A(('stu', 1)); A(('scan1', 1)); A(('gelu1', 0))
        i0 = 2
    elif start == 7:
        A(('S', 'x0', '|', 'x1', '|') + V + ('|', 'bre', '|', last, '|', 'bim', '|', 'w1'))
        A(('W', 'x0')); A(('ln1', 0)); A(('W', 'x1') + V); A(('ln1', 1))
        A(('W', 'bre')); A(('mbre', 0)); A(('lam',)); A(('mbre', 1))
        A(('W', 'bim', last)); A(('S', 'x2', '|', 'x3')); A(('mbim', 0)); A(('ln1', NT - 1)); A(('mbim', 1)); A(('stu', 0)); A(('scan1', 0))
        A(('W', 'w1')); A(('S', 'cre', 'cim') + tuple('x%d' % k for k in range(4, NT - 1))); A(('mw1', NT - 1))
        A(('W', 'x2', 'x3')); A(('stu', 1)); A(('scan1', 1)); A(('ln1', 2)); A(('gelu1', NT - 1)); A(('mw1', 0))
        A(('gelu1', 0))
        i0 = 2
    elif start == 8:
        A(('S', 'x0', '|', 'x1', '|') + V + ('|', 'bre', '|', last, '|', 'bim', '|', 'w1', '|', 'x2'))
        A(('W', 'x0')); A(('ln1', 0)); A(('W', 'x1') + V); A(('ln1', 1))
        A(('W', 'bre')); A(('mbre', 0)); A(('lam',)); A(('mbre', 1))
        A(('W', 'bim', last)); A(('mbim', 0)); A(('ln1', NT - 1)); A(('mbim', 1)); A(('stu', 0)); A(('scan1', 0))
        A(('W', 'w1', 'x2')); A(('S', 'cre', 'cim') + tuple('x%d' % k for k in range(3, NT - 1))); A(('mw1', NT - 1))
        A(('stu', 1)); A(('scan1', 1)); A(('ln1', 2)); A(('gelu1', NT - 1)); A(('mw1', 0))
        A(('gelu1', 0))
        i0 = 2
    elif start == 9:
        A(('S', 'x0', '|', 'x1', '|') + V + ('|', 'bre0', '|', 'bre1', '|', 'bre2', '|', 'bre3', '|', 'bre4', '|', 'bim', '|', last, '|', 'w1', '|', 'x2'))
        A(('W', 'x0')); A(('ln1', 0)); A(('W', 'x1') + V); A(('ln1', 1))
        for k in range(5):
            A(('W', 'bre%d' % k)); A(('mbreK', 0, k))
        A(('lam',)); A(('mbre', 1))
        A(('W', 'bim')); A(('mbim', 0)); A(('W', last)); A(('ln1', NT - 1)); A(('mbim', 1)); A(('stu', 0)); A(('scan1', 0))
        A(('W', 'w1', 'x2')); A(('S', 'cre', 'cim') + tuple('x%d' % k for k in range(3, NT - 1))); A(('mw1', NT - 1))
        A(('stu', 1)); A(('scan1', 1)); A(('ln1', 2)); A(('gelu1', NT - 1)); A(('mw1', 0))
        A(('gelu1', 0))
        i0 = 2
    elif start == 10:
        A(('S', 'x0', '|') + V + ('|', 'bre0', '|', 'bre1', '|', 'x1', '|', 'bre2', '|', 'bre3', '|', 'bre4', '|', 'bim', '|', last, '|', 'w1', '|', 'x2'))
        A(('W', 'x0')); A(('ln1', 0))
        A(('W', 'bre0') + V); A(('mbreK', 0, 0))
        A(('W', 'bre1')); A(('mbreK', 0, 1))
        A(('W', 'bre2', 'x1')); A(('mbreK', 0, 2))
        A(('W', 'bre3')); A(('mbreK', 0, 3))
        A(('W', 'bre4')); A(('ln1', 1)); A(('mbreK', 0, 4))
        A(('lam',)); A(('mbre', 1))
        A(('W', 'bim')); A(('mbim', 0)); A(('W', last)); A(('ln1', NT - 1)); A(('mbim', 1)); A(('stu', 0)); A(('scan1', 0))
        A(('W', 'w1', 'x2')); A(('S', 'cre', 'cim') + tuple('x%d' % k for k in range(3, NT - 1))); A(('mw1', NT - 1))
        A(('stu', 1)); A(('scan1', 1)); A(('ln1', 2)); A(('gelu1', NT - 1)); A(('mw1', 0))
        A(('gelu1', 0))
        i0 = 2
    for t in range(i0, NT):
        A(('mbre', t))
        if t == i0:
            A(('W',) + tuple('x%d' % k for k in range({1: 2, 2: 4, 4: 5, 5: 5, 6: 4, 7: 4, 8: 3, 9: 3, 10: 3}[start], NT - 1))); A(('S', 'w2', 'w3', 'w4'))
        if t == cfg.get('cpos', 3):
            A(('W', 'cre', 'cim') + (('w2', 'w3', 'w4') if cfg.get('wbar', 5) == t else ()))
            A(('cprep',))
        elif t == cfg.get('wbar', 5):
            A(('W', 'w2', 'w3', 'w4'))
        if t + 1 < NT - 1: A(('ln1', t + 1))
        A(('mbim', t))
        if t == NT - 1 and cfg.get('hoist', 1):
            A(('halo', 0)); A(('gsel', 0)); A(('m2', 0))
        A(('mw1', t - 1))
        A(('stu', t)); A(('scan1', t)); A(('gelu1', t - 1))
    if not cfg.get('hoist', 1):
        A(('halo', 0)); A(('gsel', 0)); A(('m2', 0))
    A(('halo', 1)); A(('carry',)); A(('ln2', 0))
    body = P2[cfg.get('p2', 'I')]
    for t in range(NT):
        for op in body:
            if op == 'm3c':
                for c in range(3): A(('m3c', t, c))
            elif op == 'outc':
                for n in range(5): A(('outc', t, n))
            elif op[:-1] == 'outc':
                A(('outc', t, int(op[-1])))
            elif op.endswith('+'):
                if t + 1 < NT: A((op[:-1], t + 1))
            else:
                A((op, t))
    return prog

def make(J=32, cfg={}, scopes=False, prog=None):
    NT = L // J
    T = J * NS
    if prog is None:
        prog = default_prog(NT, cfg)
    lastchunks = 0

    def kernel(x_h, lre_h, lim_h, ldt_h, dsk_h, bre_h, bim_h, cre_h, cim_h, w1_h, w2_h, w3_h, w4_h,
               o_h,
               x_s, v0_s, v1_s, v2_s, v3_s, bre_s, bim_s, cre_s, cim_s, w1_s, w2_s, w3_s, w4_s,
               nat_s, xn_s, xp_s, ur_s, ui_s, h_s, o_s, mk_s, xsem, wsem, osem, bsem):
        class Multi:
            def __init__(self, h, s_, sem):
                self.h, self.s, self.sem = h, s_, sem
            def start(self):
                for k in range(self.s.shape[0]):
                    pltpu.make_async_copy(self.h.at[:, pl.ds(k * 128, 128)], self.s.at[k], self.sem).start()
            def wait(self):
                pltpu.make_async_copy(self.s, self.s, self.sem).wait()
        def wload(ref, rows=None, blocks=None):
            r32 = ref.bitcast(jnp.int32)
            blocks = range(ref.shape[0]) if blocks is None else blocks
            if rows is None:
                parts = [pltpu.bitcast(r32[k], bf16) for k in blocks]
            else:
                parts = [pltpu.bitcast(r32[k, pl.ds(rows[0] // 2, (rows[1] - rows[0]) // 2), :], bf16) for k in blocks]
            return jnp.concatenate(parts, axis=1) if len(parts) > 1 else parts[0]
        wc = dict(
            bre=Multi(bre_h, bre_s, wsem.at[0]),
            bim=Multi(bim_h, bim_s, wsem.at[1]),
            w1=Multi(w1_h, w1_s, wsem.at[2]),
            cre=Multi(cre_h, cre_s, wsem.at[3]),
            cim=Multi(cim_h, cim_s, wsem.at[4]),
            w2=Multi(w2_h, w2_s, wsem.at[5]),
            w3=Multi(w3_h, w3_s, wsem.at[6]),
            w4=Multi(w4_h, w4_s, wsem.at[7]),
            lre=pltpu.make_async_copy(lre_h, v0_s, wsem.at[8]),
            lim=pltpu.make_async_copy(lim_h, v1_s, wsem.at[9]),
            ldt=pltpu.make_async_copy(ldt_h, v2_s, wsem.at[10]),
            dsk=pltpu.make_async_copy(dsk_h, v3_s, wsem.at[11]),
        )
        for k in range(5):
            wc['bre%d' % k] = pltpu.make_async_copy(bre_h.at[:, pl.ds(k * 128, 128)], bre_s.at[k], wsem.at[12 + k])
        for t in range(NT):
            wc['x%d' % t] = pltpu.make_async_copy(x_h.at[:, pl.ds(t * J, J), :], x_s.at[t], xsem.at[t])
        ocs = []
        def ocopy(t, n=None):
            if n is None:
                return pltpu.make_async_copy(o_s.at[t], o_h.at[:, pl.ds(t * J, J), :], osem.at[t])
            cs = pl.ds(n * 128, 128)
            return pltpu.make_async_copy(o_s.at[t, :, :, cs], o_h.at[:, pl.ds(t * J, J), cs], osem.at[NT + n])
        st = {}
        def mark(name):
            if scopes:
                with jax.named_scope(name):
                    mk_s[0, 0] = 1

        def B_():
            pl.semaphore_signal(bsem, 1)
            pl.semaphore_wait(bsem, 1)
        def S_(*names):
            for n in names:
                if n == '|':
                    B_()
                else:
                    wc[n].start()
        def W_(*names):
            for n in names:
                wc[n].wait()
            mark('W_' + (names[0] if names else 'none'))

        def ln1(t):
            xf = x_s[t].reshape(T, D).astype(f32)
            for s_ in range(NS):
                for j0 in range(0, J, 8):
                    for c in range(5):
                        nat_s[t, c, pl.ds(j0 * 9 + s_, 8, stride=9), :] = xf[s_ * J + j0: s_ * J + j0 + 8, c * 128:(c + 1) * 128]
            xs = [jnp.concatenate([nat_s[t, c, pl.ds(j * 9, NS), :] for c in range(5)], axis=1) for j in range(J)]
            x = jnp.concatenate(xs, axis=0)
            m = jnp.mean(x, axis=-1, keepdims=True)
            xc = x - m
            v = jnp.mean(xc * xc, axis=-1, keepdims=True)
            rs = lax.rsqrt(v + EPS)
            xn = xc * rs
            k2 = lax.rsqrt(v * rs * rs + EPS)
            xn_s[pl.ds(t * T, T), :] = xn
            xp_s[pl.ds(t * T, T), :] = x
            st['xb', t] = xn.astype(bf16)
            st['k2', t] = k2

        def mw1(t):
            st['z', t] = jnp.dot(st['xb', t], wload(w1_s), preferred_element_type=f32)

        def gelu1(t):
            z = st['z', t] * st['k2', t]
            u = z * (C0 + (C0 * C1) * (z * z))
            h_s[pl.ds(t * T + 16, T), :] = (0.5 * z) * (1.0 + jnp.tanh(u))

        def mbre(t):
            st['ur', t] = lax.dot_general(st['xb', t], wload(bre_s), NTD, preferred_element_type=f32)

        def mbreP(t, a, b):
            st.setdefault(('urp', t), []).append(lax.dot_general(st['xb', t], wload(bre_s, (a * 128, b * 128)), NTD, preferred_element_type=f32))
            if b == 5:
                st['ur', t] = jnp.concatenate(st['urp', t], axis=1)

        def mbreK(t, k):
            part = lax.dot_general(st['xb', t][:, k * 128:(k + 1) * 128], wload(bre_s, None, [k]), NTD, preferred_element_type=f32)
            st['ur', t] = part if k == 0 else st['ur', t] + part

        def mbim(t):
            st['ui', t] = lax.dot_general(st['xb', t], wload(bim_s), NTD, preferred_element_type=f32)

        def stu(t):
            ur_s[pl.ds(t * T, T), :] = st['ur', t]
            ui_s[pl.ds(t * T, T), :] = st['ui', t]

        def scan1(t):
            lr, li = st['l']
            ur, ui = st['ur', t], st['ui', t]
            if t == 0:
                er, ei = ur[0:8], ui[0:8]
            else:
                er, ei = st['e']
            for j in range(1 if t == 0 else 0, J):
                a = ur[j * 8:(j + 1) * 8]; b = ui[j * 8:(j + 1) * 8]
                er, ei = lr * er - li * ei + a, lr * ei + li * er + b
            st['e'] = (er, ei)

        def cprep():
            cr2, ci2 = st['c2']
            c32 = cre_s.bitcast(jnp.int32); d32 = cim_s.bitcast(jnp.int32)
            for k in range(5):
                a2 = cr2[:, k * 128:(k + 1) * 128]; b2 = ci2[:, k * 128:(k + 1) * 128]
                for r in range(0, D // 2, 32):
                    cre = pltpu.bitcast(c32[k, pl.ds(r, 32), :], bf16).astype(f32)
                    cim = pltpu.bitcast(d32[k, pl.ds(r, 32), :], bf16).astype(f32)
                    o1 = cre * a2 - cim * b2
                    o2 = -(cre * b2 + cim * a2)
                    c32[k, pl.ds(r, 32), :] = pltpu.bitcast(o1.astype(bf16), jnp.int32)
                    d32[k, pl.ds(r, 32), :] = pltpu.bitcast(o2.astype(bf16), jnp.int32)

        def lam():
            lre = v0_s[...].astype(f32).reshape(1, P)
            lim = v1_s[...].astype(f32).reshape(1, P)
            dt = jnp.exp(v2_s[...].astype(f32)).astype(bf16).astype(f32).reshape(1, P)
            mag = jnp.exp(dt * lre)
            lr1 = mag * jnp.cos(dt * lim)
            li1 = mag * jnp.sin(dt * lim)
            den = lre * lre + lim * lim
            nr = lr1 - 1.0
            cr2 = 2.0 * (nr * lre + li1 * lim) / den
            ci2 = 2.0 * (li1 * lre - nr * lim) / den
            st['l'] = (jnp.broadcast_to(lr1, (8, P)), jnp.broadcast_to(li1, (8, P)))
            st['c2'] = (cr2, ci2)

        sub = lax.broadcasted_iota(jnp.int32, (8, P), 0)
        col = lax.broadcasted_iota(jnp.int32, (1, D), 1)

        def halo(side):
            for k in range(2):
                if side == 0:
                    src = h_s[pl.ds(16 + (L - 2 + k) * 8, 8), :]
                    h_s[pl.ds(k * 8, 8), :] = jnp.where(sub >= 1, pltpu.roll(src, 1, 0), 0.0)
                else:
                    src = h_s[pl.ds(16 + k * 8, 8), :]
                    h_s[pl.ds(16 + (L + k) * 8, 8), :] = jnp.where(sub <= 6, pltpu.roll(src, 7, 0), 0.0)

        def csq(pr, pi):
            return pr * pr - pi * pi, 2.0 * pr * pi

        def carry():
            pr, pi = st['l']
            n = 1
            er, ei = st['e']
            while n < L:
                pr, pi = csq(pr, pi); n *= 2
            for sh in (1, 2, 4):
                gr = jnp.where(sub >= sh, pltpu.roll(er, sh, 0), 0.0)
                gi = jnp.where(sub >= sh, pltpu.roll(ei, sh, 0), 0.0)
                er, ei = er + pr * gr - pi * gi, ei + pr * gi + pi * gr
                pr, pi = csq(pr, pi)
            st['h'] = (jnp.where(sub >= 1, pltpu.roll(er, 1, 0), 0.0),
                       jnp.where(sub >= 1, pltpu.roll(ei, 1, 0), 0.0))

        def gsel(t):
            r0 = t * T
            g0 = h_s[pl.ds(r0 + 8, T), :]
            g1 = h_s[pl.ds(r0 + 24, T), :]
            g2 = h_s[pl.ds(r0, T), :]
            g3 = h_s[pl.ds(r0 + 32, T), :]
            z = jnp.where(col < 160, g0, jnp.where(col < 320, g1, jnp.where(col < 480, g2, g3)))
            st['g', t] = z.astype(bf16)

        def m2(t):
            st['hs', t] = jnp.dot(st['g', t], wload(w2_s), preferred_element_type=f32)

        def ln2(t):
            x1 = xn_s[pl.ds(t * T, T), :] + st['hs', t]
            m = jnp.mean(x1, axis=-1, keepdims=True)
            xc = x1 - m
            v = jnp.mean(xc * xc, axis=-1, keepdims=True)
            st['x1', t] = x1
            st['l2', t] = (xc * lax.rsqrt(v + EPS)).astype(bf16)

        def scan2(t):
            hr, hi = st['h']
            lr, li = st['l']
            ur = ur_s[pl.ds(t * T, T), :]
            ui = ui_s[pl.ds(t * T, T), :]
            hrs, his = [], []
            for j in range(J):
                a = ur[j * 8:(j + 1) * 8]; b = ui[j * 8:(j + 1) * 8]
                hr, hi = lr * hr - li * hi + a, lr * hi + li * hr + b
                hrs.append(hr); his.append(hi)
            st['h'] = (hr, hi)
            st['hrb', t] = jnp.concatenate(hrs, axis=0).astype(bf16)
            st['hib', t] = jnp.concatenate(his, axis=0).astype(bf16)

        def m3(t):
            z = jnp.dot(st['l2', t], wload(w3_s), preferred_element_type=f32)
            u = z * (C0 + (C0 * C1) * (z * z))
            st['a', t] = ((0.5 * z) * (1.0 + jnp.tanh(u))).astype(bf16)

        def mc(t):
            st['dsk'] = v3_s[...].astype(f32).reshape(1, D)
            s1 = lax.dot_general(st['hrb', t], wload(cre_s), NTD, preferred_element_type=f32)
            s2 = lax.dot_general(st['hib', t], wload(cim_s), NTD, preferred_element_type=f32)
            st['s', t] = s1 + s2 + xn_s[pl.ds(t * T, T), :] * st['dsk']

        def m4(t):
            st['y4', t] = jnp.dot(st['a', t], wload(w4_s), preferred_element_type=f32)

        def fin(t):
            if t == NT - 1 and cfg.get('tail', 4) > 1:
                nq = cfg.get('tail', 4)
                jq = J // nq
                for q in range(nq):
                    rs_ = slice(q * jq * 8, (q + 1) * jq * 8)
                    x2 = st['x1', t][rs_] + st['y4', t][rs_]
                    gate = x2 * jax.nn.sigmoid(x2)
                    out = xp_s[pl.ds(t * T + q * jq * 8, jq * 8), :] + st['s', t][rs_] * gate
                    for j in range(jq):
                        for c in range(5):
                            nat_s[t, c, pl.ds((q * jq + j) * 9, NS), :] = out[j * 8:(j + 1) * 8, c * 128:(c + 1) * 128]
                    for s_ in range(NS):
                        for j0 in range(q * jq, (q + 1) * jq, 8):
                            o_s[t, s_, pl.ds(j0, 8), :] = jnp.concatenate(
                                [nat_s[t, c, pl.ds(j0 * 9 + s_, 8, stride=9), :] for c in range(5)], axis=1)
                    c = pltpu.make_async_copy(o_s.at[t, :, pl.ds(q * jq, jq), :], o_h.at[:, pl.ds(t * J + q * jq, jq), :], osem.at[NT + q])
                    c.start(); ocs.append(c)
                st['done', t] = True
                return
            x2 = st['x1', t] + st['y4', t]
            gate = x2 * jax.nn.sigmoid(x2)
            out = xp_s[pl.ds(t * T, T), :] + st['s', t] * gate
            for j in range(J):
                for c in range(5):
                    nat_s[t, c, pl.ds(j * 9, NS), :] = out[j * 8:(j + 1) * 8, c * 128:(c + 1) * 128]
            for s_ in range(NS):
                for j0 in range(0, J, 8):
                    o_s[t, s_, pl.ds(j0, 8), :] = jnp.concatenate(
                        [nat_s[t, c, pl.ds(j0 * 9 + s_, 8, stride=9), :] for c in range(5)], axis=1)

        def m3c(t, c):
            z = jnp.dot(st['l2', t], wload(w3_s, None, range(c * 4, c * 4 + 4)), preferred_element_type=f32)
            u = z * (C0 + (C0 * C1) * (z * z))
            st['a', t, c] = ((0.5 * z) * (1.0 + jnp.tanh(u))).astype(bf16)

        def outd(t, n):
            cs = slice(n * 128, (n + 1) * 128)
            if ('a', t) not in st:
                st['a', t] = jnp.concatenate([st['a', t, c] for c in range(3)], axis=1)
            y4 = jnp.dot(st['a', t], wload(w4_s, None, [n]), preferred_element_type=f32)
            s1 = lax.dot_general(st['hrb', t], wload(cre_s, (n * 128, n * 128 + 128)), NTD, preferred_element_type=f32)
            s2 = lax.dot_general(st['hib', t], wload(cim_s, (n * 128, n * 128 + 128)), NTD, preferred_element_type=f32)
            st['od', t, n] = (y4, s1, s2)

        def outf(t, n):
            cs = slice(n * 128, (n + 1) * 128)
            st['dsk'] = v3_s[...].astype(f32).reshape(1, D)
            y4, s1, s2 = st['od', t, n]
            sv = s1 + s2 + xn_s[pl.ds(t * T, T), cs] * st['dsk'][:, cs]
            x2 = st['x1', t][:, cs] + y4
            gate = x2 * jax.nn.sigmoid(x2)
            out = xp_s[pl.ds(t * T, T), cs] + sv * gate
            for j in range(J):
                nat_s[t, n, pl.ds(j * 9, NS), :] = out[j * 8:(j + 1) * 8]
            for s_ in range(NS):
                for j0 in range(0, J, 8):
                    o_s[t, s_, pl.ds(j0, 8), cs] = nat_s[t, n, pl.ds(j0 * 9 + s_, 8, stride=9), :]

        def outs(t, n):
            c = ocopy(t, n); c.start(); ocs.append(c)
            st['done', t] = True

        def outc(t, n):
            outd(t, n)
            if t == NT - 1 and cfg.get('tailc', 1):
                if n > 0: outs(t, n - 1)
                outf(t, n)
                if n == 4: outs(t, 4)
            else:
                outf(t, n)

        def ost(t):
            if ('done', t) not in st:
                c = ocopy(t); c.start(); ocs.append(c)
            mark('o%d' % t)

        fns = dict(mbreK=mbreK, mbreP=mbreP, B=B_, m3c=m3c, outc=outc, ost=ost, S=S_, W=W_, ln1=ln1, mw1=mw1, gelu1=gelu1, mbre=mbre, mbim=mbim, stu=stu, scan1=scan1, cprep=cprep,
                   lam=lam, halo=halo, carry=carry, gsel=gsel, m2=m2, ln2=ln2, scan2=scan2, m3=m3, mc=mc, m4=m4, fin=fin)
        for op in prog:
            fns[op[0]](*op[1:])
        for c in ocs:
            c.wait()
        mark('end')

    def run(A_x, A_Lambda_re, A_Lambda_im, A_B_re, A_B_im, A_C_re, A_C_im, A_log_dt, A_Dskip, B_x, B_w1, B_w2, B_w3, B_w4):
        x = A_x.reshape(NS, L, D)
        hbm = pl.BlockSpec(memory_space=pl.ANY)
        out = pl.pallas_call(
            kernel,
            in_specs=[hbm] * 13,
            out_specs=hbm,
            out_shape=jax.ShapeDtypeStruct((NS, L, D), f32),
            scratch_shapes=[
                pltpu.VMEM((NT, NS, J, D), bf16),
                pltpu.VMEM((D,), bf16), pltpu.VMEM((D,), bf16), pltpu.VMEM((D,), bf16), pltpu.VMEM((D,), bf16),
                pltpu.VMEM((5, P, 128), bf16), pltpu.VMEM((5, P, 128), bf16),
                pltpu.VMEM((5, D, 128), bf16), pltpu.VMEM((5, D, 128), bf16),
                pltpu.VMEM((5, D, 128), bf16), pltpu.VMEM((5, D, 128), bf16),
                pltpu.VMEM((12, D, 128), bf16), pltpu.VMEM((5, F, 128), bf16),
                pltpu.VMEM((NT, 5, J * 9, 128), f32),
                pltpu.VMEM((S, D), f32), pltpu.VMEM((S, D), f32),
                pltpu.VMEM((S, P), f32), pltpu.VMEM((S, P), f32),
                pltpu.VMEM((S + 32, D), f32),
                pltpu.VMEM((NT, NS, J, D), f32),
                pltpu.SMEM((1, 1), jnp.int32),
                pltpu.SemaphoreType.DMA((NT,)),
                pltpu.SemaphoreType.DMA((20,)),
                pltpu.SemaphoreType.DMA((NT + 5,)),
                pltpu.SemaphoreType.REGULAR,
            ],
            compiler_params=pltpu.CompilerParams(vmem_limit_bytes=110 * 1024 * 1024,
                flags=({'XLA_TPU_EVENLY_DISTRIBUTE_CRITICAL_NODES': True} if cfg.get('even', 1) else None)),
        )(x, A_Lambda_re, A_Lambda_im, A_log_dt, A_Dskip, A_B_re, A_B_im, A_C_re, A_C_im, B_w1, B_w2, B_w3, B_w4)
        return out.reshape(1, S, D)
    return jax.jit(run)


_FN = make(32, {'p2': 'I', 'cpos': 5, 'start': 8})


@jax.jit
def pallas_recurrent_scan__ssm_conv_s5__mixer_s_mlp__prompt_kernel(
    A_x, A_Lambda_re, A_Lambda_im, A_B_re, A_B_im, A_C_re, A_C_im,
    A_log_dt, A_Dskip, B_x, B_w1, B_w2, B_w3, B_w4,
):
    return _FN(A_x, A_Lambda_re, A_Lambda_im, A_B_re, A_B_im, A_C_re, A_C_im,
               A_log_dt, A_Dskip, B_x, B_w1, B_w2, B_w3, B_w4)
```

```python
import jax
import jax.numpy as jnp
from jax import lax
from jax.experimental import pallas as pl
from jax.experimental.pallas import tpu as pltpu

S, D, P, F = 2048, 640, 640, 1536
NS = 8
L = S // NS
J = 32
NT = L // J
T = J * NS
NB = D // 128
EPS = 1e-5
f32, bf16, i32 = jnp.float32, jnp.bfloat16, jnp.int32
C0 = 0.7978845608028654
C1 = 0.044715
NTD = (((1,), (1,)), ((), ()))


def _dot(a, b):
    return jnp.dot(a, b, preferred_element_type=f32)


def _dot_nt(a, b):
    return lax.dot_general(a, b, NTD, preferred_element_type=f32)


def _gelu(z):
    u = z * (C0 + (C0 * C1) * (z * z))
    return (0.5 * z) * (1.0 + jnp.tanh(u))


def _cmul_add(lr, li, hr, hi, a, b):
    return lr * hr - li * hi + a, lr * hi + li * hr + b


def _csq(pr, pi):
    return pr * pr - pi * pi, 2.0 * pr * pi


class _Blocked:
    def __init__(self, src, dst, sem, rows=None):
        self.src, self.dst, self.sem = src, dst, sem
        self.rows = rows if rows is not None else pl.ds(0, src.shape[0])

    def start(self):
        for k in range(self.dst.shape[0]):
            pltpu.make_async_copy(self.src.at[self.rows, pl.ds(k * 128, 128)],
                                  self.dst.at[k, self.rows, :], self.sem).start()

    def wait(self):
        v = self.dst.at[:, self.rows, :]
        pltpu.make_async_copy(v, v, self.sem).wait()


def _wload(ref, rows=None, blocks=None):
    r32 = ref.bitcast(i32)
    blocks = range(ref.shape[0]) if blocks is None else blocks
    if rows is None:
        parts = [pltpu.bitcast(r32[k], bf16) for k in blocks]
    else:
        sl = pl.ds(rows[0] // 2, (rows[1] - rows[0]) // 2)
        parts = [pltpu.bitcast(r32[k, sl, :], bf16) for k in blocks]
    return jnp.concatenate(parts, axis=1) if len(parts) > 1 else parts[0]


def _kernel(x_h, lre_h, lim_h, ldt_h, dsk_h, bre_h, bim_h, cre_h, cim_h, w1_h, w2_h, w3_h, w4_h,
            o_h,
            x_s, lre_s, lim_s, ldt_s, dsk_s, bre_s, bim_s, cre_s, cim_s, w1_s, w2_s, w3_s, w4_s,
            perm_s, xn_s, xp_s, ur_s, ui_s, h_s, o_s, xsem, wsem, osem, bsem):
    cp = dict(
        bim=_Blocked(bim_h, bim_s, wsem.at[0]), w1=_Blocked(w1_h, w1_s, wsem.at[1]),
        cre=_Blocked(cre_h, cre_s, wsem.at[2]), cim=_Blocked(cim_h, cim_s, wsem.at[3]),
        w2=_Blocked(w2_h, w2_s, wsem.at[4]), w3=_Blocked(w3_h, w3_s, wsem.at[5]),
        w4=_Blocked(w4_h, w4_s, wsem.at[6]),
        lre=pltpu.make_async_copy(lre_h, lre_s, wsem.at[7]),
        lim=pltpu.make_async_copy(lim_h, lim_s, wsem.at[8]),
        ldt=pltpu.make_async_copy(ldt_h, ldt_s, wsem.at[9]),
        dsk=pltpu.make_async_copy(dsk_h, dsk_s, wsem.at[10]),
    )
    for n in range(NB):
        cp['bre%d' % n] = _Blocked(bre_h, bre_s, wsem.at[11 + n], pl.ds(n * 128, 128))
    for t in range(NT):
        cp['x%d' % t] = pltpu.make_async_copy(x_h.at[:, pl.ds(t * J, J), :], x_s.at[t], xsem.at[t])
    out_copies = []
    st = {}

    def start(*names):
        for n in names:
            if n == '|':
                pl.semaphore_signal(bsem, 1)
                pl.semaphore_wait(bsem, 1)
            else:
                cp[n].start()

    def wait(*names):
        for n in names:
            cp[n].wait()

    sub = lax.broadcasted_iota(i32, (8, P), 0)
    col = lax.broadcasted_iota(i32, (1, D), 1)

    def ln1(t):
        xf = x_s[t].reshape(T, D).astype(f32)
        for s_ in range(NS):
            for j0 in range(0, J, 8):
                for c in range(NB):
                    perm_s[t, c, pl.ds(j0 * 9 + s_, 8, stride=9), :] = (
                        xf[s_ * J + j0:s_ * J + j0 + 8, c * 128:(c + 1) * 128])
        x = jnp.concatenate(
            [jnp.concatenate([perm_s[t, c, pl.ds(j * 9, NS), :] for c in range(NB)], axis=1)
             for j in range(J)], axis=0)
        m = jnp.mean(x, axis=-1, keepdims=True)
        xc = x - m
        v = jnp.mean(xc * xc, axis=-1, keepdims=True)
        rs = lax.rsqrt(v + EPS)
        xn = xc * rs
        st['k2', t] = lax.rsqrt(v * rs * rs + EPS)
        xn_s[pl.ds(t * T, T), :] = xn
        xp_s[pl.ds(t * T, T), :] = x
        st['xb', t] = xn.astype(bf16)

    def lam():
        lre = lre_s[...].astype(f32).reshape(1, P)
        lim = lim_s[...].astype(f32).reshape(1, P)
        dt = jnp.exp(ldt_s[...].astype(f32)).astype(bf16).astype(f32).reshape(1, P)
        mag = jnp.exp(dt * lre)
        lr = mag * jnp.cos(dt * lim)
        li = mag * jnp.sin(dt * lim)
        den = lre * lre + lim * lim
        nr = lr - 1.0
        st['c2'] = (2.0 * (nr * lre + li * lim) / den, 2.0 * (li * lre - nr * lim) / den)
        st['l'] = (jnp.broadcast_to(lr, (8, P)), jnp.broadcast_to(li, (8, P)))

    def mbre_part(t, a, b):
        st.setdefault(('urp', t), []).append(_dot_nt(st['xb', t], _wload(bre_s, (a * 128, b * 128))))
        if b == NB:
            st['ur', t] = jnp.concatenate(st['urp', t], axis=1)

    def mbre(t):
        st['ur', t] = _dot_nt(st['xb', t], _wload(bre_s))

    def mbim(t):
        st['ui', t] = _dot_nt(st['xb', t], _wload(bim_s))

    def mw1(t):
        st['z', t] = _dot(st['xb', t], _wload(w1_s))

    def gelu1(t):
        h_s[pl.ds(t * T + 16, T), :] = _gelu(st['z', t] * st['k2', t])

    def stu(t):
        ur_s[pl.ds(t * T, T), :] = st['ur', t]
        ui_s[pl.ds(t * T, T), :] = st['ui', t]

    def scan1(t):
        lr, li = st['l']
        ur, ui = st['ur', t], st['ui', t]
        er, ei = (ur[0:8], ui[0:8]) if t == 0 else st['e']
        for j in range(1 if t == 0 else 0, J):
            er, ei = _cmul_add(lr, li, er, ei, ur[j * 8:(j + 1) * 8], ui[j * 8:(j + 1) * 8])
        st['e'] = (er, ei)

    def carry():
        er, ei = st['e']
        pr, pi = st['l']
        n = 1
        while n < L:
            pr, pi = _csq(pr, pi)
            n *= 2
        for sh in (1, 2, 4):
            gr = jnp.where(sub >= sh, pltpu.roll(er, sh, 0), 0.0)
            gi = jnp.where(sub >= sh, pltpu.roll(ei, sh, 0), 0.0)
            er, ei = er + pr * gr - pi * gi, ei + pr * gi + pi * gr
            pr, pi = _csq(pr, pi)
        st['h'] = (jnp.where(sub >= 1, pltpu.roll(er, 1, 0), 0.0),
                   jnp.where(sub >= 1, pltpu.roll(ei, 1, 0), 0.0))

    def cprep():
        cr2, ci2 = st['c2']
        c32, d32 = cre_s.bitcast(i32), cim_s.bitcast(i32)
        for k in range(NB):
            a2, b2 = cr2[:, k * 128:(k + 1) * 128], ci2[:, k * 128:(k + 1) * 128]
            for r in range(0, D // 2, 32):
                cre = pltpu.bitcast(c32[k, pl.ds(r, 32), :], bf16).astype(f32)
                cim = pltpu.bitcast(d32[k, pl.ds(r, 32), :], bf16).astype(f32)
                c32[k, pl.ds(r, 32), :] = pltpu.bitcast((cre * a2 - cim * b2).astype(bf16), i32)
                d32[k, pl.ds(r, 32), :] = pltpu.bitcast((-(cre * b2 + cim * a2)).astype(bf16), i32)

    def halo(side):
        for k in range(2):
            if side == 0:
                src = h_s[pl.ds(16 + (L - 2 + k) * 8, 8), :]
                h_s[pl.ds(k * 8, 8), :] = jnp.where(sub >= 1, pltpu.roll(src, 1, 0), 0.0)
            else:
                src = h_s[pl.ds(16 + k * 8, 8), :]
                h_s[pl.ds(16 + (L + k) * 8, 8), :] = jnp.where(sub <= 6, pltpu.roll(src, 7, 0), 0.0)

    def m2(t):
        r0 = t * T
        g0 = h_s[pl.ds(r0 + 8, T), :]
        g1 = h_s[pl.ds(r0 + 24, T), :]
        g2 = h_s[pl.ds(r0, T), :]
        g3 = h_s[pl.ds(r0 + 32, T), :]
        c = D // 4
        g = jnp.where(col < c, g0, jnp.where(col < 2 * c, g1, jnp.where(col < 3 * c, g2, g3)))
        st['hs', t] = _dot(g.astype(bf16), _wload(w2_s))

    def ln2(t):
        x1 = xn_s[pl.ds(t * T, T), :] + st['hs', t]
        m = jnp.mean(x1, axis=-1, keepdims=True)
        xc = x1 - m
        v = jnp.mean(xc * xc, axis=-1, keepdims=True)
        st['x1', t] = x1
        st['l2', t] = (xc * lax.rsqrt(v + EPS)).astype(bf16)

    def scan2(t):
        hr, hi = st['h']
        lr, li = st['l']
        ur = ur_s[pl.ds(t * T, T), :]
        ui = ui_s[pl.ds(t * T, T), :]
        hrs, his = [], []
        for j in range(J):
            hr, hi = _cmul_add(lr, li, hr, hi, ur[j * 8:(j + 1) * 8], ui[j * 8:(j + 1) * 8])
            hrs.append(hr)
            his.append(hi)
        st['h'] = (hr, hi)
        st['hrb', t] = jnp.concatenate(hrs, axis=0).astype(bf16)
        st['hib', t] = jnp.concatenate(his, axis=0).astype(bf16)

    def m3(t, c):
        st['a', t, c] = _gelu(_dot(st['l2', t], _wload(w3_s, None, range(c * 4, c * 4 + 4)))).astype(bf16)

    def out_copy(t, n=None):
        rows = pl.ds(t * J, J)
        if n is None:
            c = pltpu.make_async_copy(o_s.at[t], o_h.at[:, rows, :], osem.at[t])
        else:
            cs = pl.ds(n * 128, 128)
            c = pltpu.make_async_copy(o_s.at[t, :, :, cs], o_h.at[:, rows, cs], osem.at[NT + n])
        c.start()
        out_copies.append(c)

    def outc(t, n):
        cs = slice(n * 128, (n + 1) * 128)
        rows = (n * 128, n * 128 + 128)
        y4 = None
        for c in range(3):
            p_ = _dot(st['a', t, c], _wload(w4_s, (c * 512, c * 512 + 512), [n]))
            y4 = p_ if y4 is None else y4 + p_
        s1 = _dot_nt(st['hrb', t], _wload(cre_s, rows))
        s2 = _dot_nt(st['hib', t], _wload(cim_s, rows))
        last = t == NT - 1
        if last and n > 0:
            out_copy(t, n - 1)
        dsk = dsk_s[...].astype(f32).reshape(1, D)
        sv = s1 + s2 + xn_s[pl.ds(t * T, T), cs] * dsk[:, cs]
        hx = 0.5 * (st['x1', t][:, cs] + y4)
        gate = hx + hx * jnp.tanh(hx)
        out = xp_s[pl.ds(t * T, T), cs] + sv * gate
        for j in range(J):
            perm_s[t, n, pl.ds(j * 9, NS), :] = out[j * 8:(j + 1) * 8]
        for s_ in range(NS):
            for j0 in range(0, J, 8):
                o_s[t, s_, pl.ds(j0, 8), cs] = perm_s[t, n, pl.ds(j0 * 9 + s_, 8, stride=9), :]
        if last and n == NB - 1:
            out_copy(t, n)

    vec = ('lre', 'lim', 'ldt', 'dsk')
    xl = 'x%d' % (NT - 1)
    start('x0', '|', *vec, '|', 'bre0', '|', 'bre1', '|', 'bre2', '|', 'x1', '|', 'bre3', '|', 'bre4',
          '|', 'bim', '|', xl, '|', 'w1', '|', 'x2')
    wait('x0'); ln1(0)
    wait('bre0', 'bre1', *vec); mbre_part(0, 0, 2); lam()
    wait('x1', 'bre2'); mbre_part(0, 2, 3); ln1(1)
    wait('bre3', 'bre4'); mbre_part(0, 3, 5)
    mbre(1)
    wait('bim', xl); mbim(0); ln1(NT - 1); mbim(1); stu(0); scan1(0)
    wait('w1', 'x2'); start('cre', 'cim', *['x%d' % k for k in range(3, NT - 1)]); mw1(NT - 1)
    stu(1); scan1(1); ln1(2); gelu1(NT - 1); mw1(0); gelu1(0)
    for t in range(2, NT):
        mbre(t)
        if t == 2:
            wait(*['x%d' % k for k in range(3, NT - 1)]); start('w2', 'w3', 'w4')
        if t == 5:
            wait('cre', 'cim', 'w2', 'w3', 'w4'); cprep()
        if t + 1 < NT - 1:
            ln1(t + 1)
        mbim(t)
        if t == NT - 1:
            halo(0); m2(0)
        mw1(t - 1)
        stu(t); scan1(t); gelu1(t - 1)
    halo(1); carry(); ln2(0)
    for t in range(NT):
        for c in range(3):
            m3(t, c)
        scan2(t)
        outc(t, 0)
        if t + 1 < NT:
            m2(t + 1)
        outc(t, 1)
        if t + 1 < NT:
            ln2(t + 1)
        for n in range(2, NB):
            outc(t, n)
        if t < NT - 1:
            out_copy(t)
    for c in out_copies:
        c.wait()


@jax.jit
def pallas_recurrent_scan__ssm_conv_s5__mixer_s_mlp__prompt_kernel(
    A_x, A_Lambda_re, A_Lambda_im, A_B_re, A_B_im, A_C_re, A_C_im,
    A_log_dt, A_Dskip, B_x, B_w1, B_w2, B_w3, B_w4,
):
    del B_x
    hbm = pl.BlockSpec(memory_space=pl.ANY)
    blk = lambda nb, rows: pltpu.VMEM((nb, rows, 128), bf16)
    out = pl.pallas_call(
        _kernel,
        in_specs=[hbm] * 13,
        out_specs=hbm,
        out_shape=jax.ShapeDtypeStruct((NS, L, D), f32),
        scratch_shapes=[
            pltpu.VMEM((NT, NS, J, D), bf16),
            pltpu.VMEM((D,), bf16), pltpu.VMEM((D,), bf16), pltpu.VMEM((D,), bf16), pltpu.VMEM((D,), bf16),
            blk(NB, P), blk(NB, P), blk(NB, D), blk(NB, D), blk(NB, D), blk(NB, D),
            blk(F // 128, D), blk(NB, F),
            pltpu.VMEM((NT, NB, J * 9, 128), f32),
            pltpu.VMEM((S, D), f32), pltpu.VMEM((S, D), f32),
            pltpu.VMEM((S, P), f32), pltpu.VMEM((S, P), f32),
            pltpu.VMEM((S + 32, D), f32),
            pltpu.VMEM((NT, NS, J, D), f32),
            pltpu.SemaphoreType.DMA((NT,)),
            pltpu.SemaphoreType.DMA((16,)),
            pltpu.SemaphoreType.DMA((NT + NB,)),
            pltpu.SemaphoreType.REGULAR,
        ],
        compiler_params=pltpu.CompilerParams(
            vmem_limit_bytes=110 * 1024 * 1024,
            flags={'XLA_TPU_EVENLY_DISTRIBUTE_CRITICAL_NODES': True}),
    )(A_x.reshape(NS, L, D), A_Lambda_re, A_Lambda_im, A_log_dt, A_Dskip, A_B_re, A_B_im,
      A_C_re, A_C_im, B_w1, B_w2, B_w3, B_w4)
    return out.reshape(1, S, D)
```
